```python
import os as _os
_os.environ.setdefault("JAX_PLATFORMS", "cpu")
import jax
import jax.numpy as jnp

def _softmax(x, axis=-1):
    return jax.nn.softmax(x, axis=axis)
def _gelu(x):
    return jax.nn.gelu(x, approximate=True)
def _silu(x):
    return jax.nn.silu(x)
def _sigmoid(x):
    return jax.nn.sigmoid(x)
def _layernorm(x, axis=-1, eps=1e-5):
    m = jnp.mean(x, axis=axis, keepdims=True)
    v = jnp.var(x, axis=axis, keepdims=True)
    return (x - m) / jnp.sqrt(v + eps)
def _scatter_add(tgt, idx, src, axis=0):
    return tgt.at[idx].add(src)
def _segment_sum(src, seg, n):
    return jax.ops.segment_sum(src, seg, n)
class _Rng:
    def __init__(self, key):
        self._k = key
    def _next(self):
        self._k, sub = jax.random.split(self._k)
        return sub
    def normal(self, shape):
        return jax.random.normal(self._next(), shape, dtype=jnp.bfloat16)
    def randint(self, lo, hi, shape):
        return jax.random.randint(self._next(), shape, lo, hi, dtype=jnp.int32)
    def uniform(self, shape, lo=0.0, hi=1.0):
        return jax.random.uniform(self._next(), shape, jnp.bfloat16, lo, hi)
    def permutation(self, n):
        return jax.random.permutation(self._next(), n)


kernel_name = 'concat_heads__mha_block_cached__gqa_block_cached__near_ridge'

def setup_inputs():
    _rng = _Rng(jax.random.key(int.from_bytes(__import__("os").urandom(4), "little")))
    _w = (lambda a: (lambda t: t.astype(jnp.bfloat16) if jnp.issubdtype(t.dtype, jnp.floating) else t)(jnp.asarray(a)))
    def _A_setup():
        B, Sq, D = 8, 128, 512
        H, Sk, Dh = 32, 1024, 128
        return {
            "x": _w((lambda *s: _rng.normal(s) * 0.8)(B, Sq, D)),
            "k_cache": _w((lambda *s: _rng.normal(s) * 0.8)(B, H, Sk, Dh)),
            "v_cache": _w((lambda *s: _rng.normal(s) * 0.05)(B, H, Sk, Dh)),
            "wq": _w((lambda *s: _rng.normal(s) * 0.8)(D, H * Dh) * (D ** -0.5)),
            "wo": _w((lambda *s: _rng.normal(s) * 0.05)(H * Dh, D) * ((H * Dh) ** -0.5)),
        }
    _A_in = _A_setup()

    def _B_setup():
        B, Sq, D = 8, 128, 512
        Hq, Hkv, Sk, Dh = 32, 32, 1024, 128
        assert Hq % Hkv == 0, (Hq, Hkv)
        return {
            "x": _w((lambda *s: _rng.normal(s) * 0.8)(B, Sq, D)),
            "k_cache": _w((lambda *s: _rng.normal(s) * 0.8)(B, Hkv, Sk, Dh)),
            "v_cache": _w((lambda *s: _rng.normal(s) * 0.05)(B, Hkv, Sk, Dh)),
            "wq": _w((lambda *s: _rng.normal(s) * 0.8)(D, Hq * Dh) * (D ** -0.5)),
            "wo": _w((lambda *s: _rng.normal(s) * 0.05)(Hq * Dh, D) * ((Hq * Dh) ** -0.5)),
        }
    _B_in = _B_setup()

    return {
        "A_x": _A_in["x"],
        "A_k_cache": _A_in["k_cache"],
        "A_v_cache": _A_in["v_cache"],
        "A_wq": _A_in["wq"],
        "A_wo": _A_in["wo"],
        "B_x": _B_in["x"],
        "B_k_cache": _B_in["k_cache"],
        "B_v_cache": _B_in["v_cache"],
        "B_wq": _B_in["wq"],
        "B_wo": _B_in["wo"],
    }

def reference(A_x, A_k_cache, A_v_cache, A_wq, A_wo, B_x, B_k_cache, B_v_cache, B_wq, B_wo):
    def _A_ref(x, k_cache, v_cache, wq, wo):
        B, Sq, D = x.shape
        H, Dh = 32, 128
        q = (lambda x, *d: x.transpose(*d))((x @ wq).reshape(B, Sq, H, Dh), 0, 2, 1, 3)
        scores = jnp.einsum("bhqd,bhkd->bhqk", q, k_cache) * (Dh ** -0.5)
        p = _softmax(scores, axis=-1)
        o = jnp.einsum("bhqk,bhkd->bhqd", p, v_cache)
        return (lambda x, *d: x.transpose(*d))(o, 0, 2, 1, 3).reshape(B, Sq, H * Dh) @ wo

    def _B_ref(x, k_cache, v_cache, wq, wo):
        B, Sq, D = x.shape
        Hq, Dh = 32, 128
        Hkv = k_cache.shape[1]
        rep = Hq // Hkv
        q = (lambda x, *d: x.transpose(*d))((x @ wq).reshape(B, Sq, Hq, Dh), 0, 2, 1, 3)
        k = jnp.repeat(k_cache, rep, axis=1)
        v = jnp.repeat(v_cache, rep, axis=1)
        scores = jnp.einsum("bhqd,bhkd->bhqk", q, k) * (Dh ** -0.5)
        p = _softmax(scores, axis=-1)
        o = jnp.einsum("bhqk,bhkd->bhqd", p, v)
        return (lambda x, *d: x.transpose(*d))(o, 0, 2, 1, 3).reshape(B, Sq, Hq * Dh) @ wo

    a = _A_ref(A_x, A_k_cache, A_v_cache, A_wq, A_wo)
    b = _B_ref(B_x, B_k_cache, B_v_cache, B_wq, B_wo)
    return jnp.concatenate([a, b], axis=-1)
```

```python
import math

import jax
import jax.numpy as jnp
from jax import lax
import jax.experimental.pallas as pl
import jax.experimental.pallas.tpu as pltpu

H, DH = 32, 128
NB = 2
C = (DH ** -0.5) * math.log2(math.e)


def _kernel(ax, ak, av, awq, awo, bx, bk, bv, bwq, bwo, o_hbm,
            xbuf, kbuf, vbuf, wqbuf, wobuf, qs, os_, acc, obuf,
            ksem, vsem, wsem, xsem, osem):
    _, B, SQ, D = xbuf.shape
    G = B // NB
    R = NB * SQ
    srcs = [(ak, av, awq, awo), (bk, bv, bwq, bwo)]
    xcp = [pltpu.make_async_copy(x, xbuf.at[j], xsem.at[j]) for j, x in enumerate((ax, bx))]

    def ocp(j, g):
        rows = pl.ds(g * NB, NB)
        return pltpu.make_async_copy(
            obuf.at[j, rows], o_hbm.at[rows, :, pl.ds(j * D, D)], osem.at[j, g])

    def wcps(j, h, slot):
        cols = pl.ds(pl.multiple_of(h * DH, DH), DH)
        return [
            pltpu.make_async_copy(srcs[j][2].at[:, cols], wqbuf.at[slot], wsem.at[0, slot]),
            pltpu.make_async_copy(srcs[j][3].at[cols, :], wobuf.at[slot], wsem.at[1, slot]),
        ]

    def kvcps(j, h, g):
        rows = pl.ds(g * NB, NB)
        return [
            pltpu.make_async_copy(srcs[j][0].at[rows, h], kbuf.at[g], ksem.at[g]),
            pltpu.make_async_copy(srcs[j][1].at[rows, h], vbuf.at[g], vsem.at[g]),
        ]

    def start(cs):
        for c in cs:
            c.start()

    def wait(cs):
        for c in cs:
            c.wait()

    xcp[0].start()
    start(wcps(0, 0, 0))
    for g in range(G):
        start(kvcps(0, 0, g))
    xcp[1].start()

    for j in range(2):
        acc[...] = jnp.zeros_like(acc)
        xcp[j].wait()

        def body(h, _):
            wslot = h % 2
            wait(wcps(j, h, wslot))
            pl.when(h + 1 < H)(lambda: start(wcps(j, h + 1, 1 - wslot)))
            if j == 0:
                pl.when(h + 1 == H)(lambda: start(wcps(1, 0, 1 - wslot)))

            q = jnp.dot(xbuf[j].reshape(B * SQ, D), wqbuf[wslot],
                        preferred_element_type=jnp.float32)
            qs[...] = (q * C).astype(jnp.bfloat16)

            for g in range(G):
                wait(kvcps(j, h, g))
                if (j, g) == (1, G - 1):
                    pl.when(h == H - 1)(lambda: start(
                        [ocp(jj, gg) for jj in range(2) for gg in range(G)
                         if (jj, gg) != (1, G - 1)]))
                for bb in range(NB):
                    rows = pl.ds((g * NB + bb) * SQ, SQ)
                    s = lax.dot_general(qs[rows, :], kbuf[g, bb], (((1,), (1,)), ((), ())),
                                        preferred_element_type=jnp.float32)
                    m = jnp.max(s, axis=-1, keepdims=True)
                    p = jnp.exp2(s - m)
                    l = jnp.sum(p, axis=-1, keepdims=True)
                    o = jnp.dot(p.astype(jnp.bfloat16), vbuf[g, bb],
                                preferred_element_type=jnp.float32)
                    os_[rows, :] = (o * (1.0 / l)).astype(jnp.bfloat16)

                pl.when(h + 1 < H)(lambda: start(kvcps(j, h + 1, g)))
                if j == 0:
                    pl.when(h + 1 == H)(lambda: start(kvcps(1, 0, g)))

                grows = pl.ds(g * R, R)
                acc[grows, :] += jnp.dot(os_[grows, :], wobuf[wslot],
                                         preferred_element_type=jnp.float32)

                @pl.when(h == H - 1)
                def _():
                    obuf[j, pl.ds(g * NB, NB)] = (
                        acc[grows, :].astype(jnp.bfloat16).reshape(NB, SQ, D))
                    if (j, g) == (1, G - 1):
                        ocp(j, g).start()

        lax.fori_loop(0, H, body, None)

    wait([ocp(j, g) for j in range(2) for g in range(G)])


@jax.jit
def pallas_concat_heads__mha_block_cached__gqa_block_cached__near_ridge_kernel(
    A_x: jax.Array,
    A_k_cache: jax.Array,
    A_v_cache: jax.Array,
    A_wq: jax.Array,
    A_wo: jax.Array,
    B_x: jax.Array,
    B_k_cache: jax.Array,
    B_v_cache: jax.Array,
    B_wq: jax.Array,
    B_wo: jax.Array,
):
    B, SQ, D = A_x.shape
    SK = A_k_cache.shape[2]
    G = B // NB
    bf, f32 = jnp.bfloat16, jnp.float32
    return pl.pallas_call(
        _kernel,
        out_shape=jax.ShapeDtypeStruct((B, SQ, 2 * D), bf),
        in_specs=[pl.BlockSpec(memory_space=pl.ANY)] * 10,
        out_specs=pl.BlockSpec(memory_space=pl.ANY),
        scratch_shapes=[
            pltpu.VMEM((2, B, SQ, D), bf),
            pltpu.VMEM((G, NB, SK, DH), bf),
            pltpu.VMEM((G, NB, SK, DH), bf),
            pltpu.VMEM((2, D, DH), bf),
            pltpu.VMEM((2, DH, D), bf),
            pltpu.VMEM((B * SQ, DH), bf),
            pltpu.VMEM((B * SQ, DH), bf),
            pltpu.VMEM((B * SQ, D), f32),
            pltpu.VMEM((2, B, SQ, D), bf),
            pltpu.SemaphoreType.DMA((G,)),
            pltpu.SemaphoreType.DMA((G,)),
            pltpu.SemaphoreType.DMA((2, 2)),
            pltpu.SemaphoreType.DMA((2,)),
            pltpu.SemaphoreType.DMA((2, G)),
        ],
        compiler_params=pltpu.CompilerParams(
            vmem_limit_bytes=100 * 1024 * 1024,
            flags={"XLA_TPU_FORCE_LP_LLO_SCHEDULER": True},
        ),
    )(A_x, A_k_cache, A_v_cache, A_wq, A_wo, B_x, B_k_cache, B_v_cache, B_wq, B_wo)
```
